```python
import jax
import jax.numpy as jnp

def _softmax(x, axis=-1):
    return jax.nn.softmax(x, axis=axis)
def _gelu(x):
    return jax.nn.gelu(x, approximate=True)
def _silu(x):
    return jax.nn.silu(x)
def _sigmoid(x):
    return jax.nn.sigmoid(x)
def _layernorm(x, axis=-1, eps=1e-5):
    m = jnp.mean(x, axis=axis, keepdims=True)
    v = jnp.var(x, axis=axis, keepdims=True)
    return (x - m) / jnp.sqrt(v + eps)
def _scatter_add(tgt, idx, src, axis=0):
    return tgt.at[idx].add(src)
def _segment_sum(src, seg, n):
    return jax.ops.segment_sum(src, seg, n)
class _Rng:
    def __init__(self, key):
        self._k = key
    def _next(self):
        self._k, sub = jax.random.split(self._k)
        return sub
    def normal(self, shape):
        return jax.random.normal(self._next(), shape, dtype=jnp.bfloat16)
    def randint(self, lo, hi, shape):
        return jax.random.randint(self._next(), shape, lo, hi, dtype=jnp.int32)
    def uniform(self, shape, lo=0.0, hi=1.0):
        return jax.random.uniform(self._next(), shape, jnp.bfloat16, lo, hi)
    def permutation(self, n):
        return jax.random.permutation(self._next(), n)


kernel_name = 'sequential_preLN__sliding_block_cached__glu_gated_swiglu__decode'

def setup_inputs():
    _rng = _Rng(jax.random.key(int.from_bytes(__import__("os").urandom(4), "little")))
    _w = (lambda a: (lambda t: t.astype(jnp.bfloat16) if jnp.issubdtype(t.dtype, jnp.floating) else t)(jnp.asarray(a)))
    def _A_setup():
        B, Sq, D = 1, 1, 640
        Hq, Hkv, Sk, Dh = 32, 32, 32768, 192
        assert Hq % Hkv == 0, (Hq, Hkv)
        return {
            "x": _w((lambda *s: _rng.normal(s) * 0.05)(B, Sq, D)),
            "k_cache": _w((lambda *s: _rng.normal(s) * 0.05)(B, Hkv, Sk, Dh)),
            "v_cache": _w((lambda *s: _rng.normal(s) * 0.05)(B, Hkv, Sk, Dh)),
            "wq": _w((lambda *s: _rng.normal(s) * 0.05)(D, Hq * Dh) * (D ** -0.5)),
            "wo": _w((lambda *s: _rng.normal(s) * 0.05)(Hq * Dh, D) * ((Hq * Dh) ** -0.5)),
        }
    _A_in = _A_setup()

    def _B_setup():
        B, S, D, F = 1, 1, 640, 1536
        return {
            "x": _w((lambda *s: _rng.normal(s) * 0.05)(B, S, D)),
            "w1": _w((lambda *s: _rng.normal(s) * 0.05)(D, F) * (2.0 / D) ** 0.5),
            "w3": _w((lambda *s: _rng.normal(s) * 0.05)(D, F) * (2.0 / D) ** 0.5),
            "w2": _w((lambda *s: _rng.normal(s) * 0.05)(F, D) * (2.0 / F) ** 0.5),
        }
    _B_in = _B_setup()

    return {
        "A_x": _A_in["x"],
        "A_k_cache": _A_in["k_cache"],
        "A_v_cache": _A_in["v_cache"],
        "A_wq": _A_in["wq"],
        "A_wo": _A_in["wo"],
        "B_x": _B_in["x"],
        "B_w1": _B_in["w1"],
        "B_w3": _B_in["w3"],
        "B_w2": _B_in["w2"],
    }

def reference(A_x, A_k_cache, A_v_cache, A_wq, A_wo, B_x, B_w1, B_w3, B_w2):
    def _A_ref(x, k_cache, v_cache, wq, wo):
        B, Sq, D = x.shape
        Hq, Dh = 32, 192
        Hkv, Sk = k_cache.shape[1], k_cache.shape[2]
        W = min(4096, max(256, Sk // 4))
        rep = Hq // Hkv
        q = (lambda x, *d: x.transpose(*d))((x @ wq).reshape(B, Sq, Hq, Dh), 0, 2, 1, 3)
        k = jnp.repeat(k_cache[:, :, Sk - W:, :], rep, axis=1)
        v = jnp.repeat(v_cache[:, :, Sk - W:, :], rep, axis=1)
        scores = jnp.einsum("bhqd,bhkd->bhqk", q, k) * (Dh ** -0.5)
        p = _softmax(scores, axis=-1)
        o = jnp.einsum("bhqk,bhkd->bhqd", p, v)
        return (lambda x, *d: x.transpose(*d))(o, 0, 2, 1, 3).reshape(B, Sq, Hq * Dh) @ wo

    def _B_ref(x, w1, w3, w2):
        gate = jnp.einsum("bsd,df->bsf", x, w1)
        up = jnp.einsum("bsd,df->bsf", x, w3)
        h = _silu(gate) * up
        out = jnp.einsum("bsf,fd->bsd", h, w2)
        return out

    x = A_x
    h = x + _A_ref(_layernorm(x, axis=-1), A_k_cache, A_v_cache, A_wq, A_wo)
    h2 = h + _B_ref(_layernorm(h, axis=-1), B_w1, B_w3, B_w2)
    return h2
```

```python
import jax
import jax.numpy as jnp
import numpy as np
from jax import lax
import jax.experimental.pallas as pl
import jax.experimental.pallas.tpu as pltpu

H, DH, SK, D, F = 32, 192, 32768, 640, 1536
W = min(4096, max(256, SK // 4))
BF = jnp.bfloat16
F32 = jnp.float32


def _bf16_round(v):
    u = int(np.float32(v).view(np.uint32))
    u = (u + 0x7FFF + ((u >> 16) & 1)) & 0xFFFF0000
    return float(np.uint32(u).view(np.float32))


SCALE = _bf16_round(DH ** -0.5)
EPS = _bf16_round(1e-5)


def _r(x):
    return x.astype(BF).astype(F32)


def _layernorm(x32):
    m = jnp.mean(x32, axis=-1, keepdims=True)
    c = x32 - m
    v = jnp.mean(c * c, axis=-1, keepdims=True)
    num = _r(x32 - _r(m))
    den = _r(jnp.sqrt(_r(_r(v) + EPS)))
    return (num / den).astype(BF)


TILE = 128


def _rects(tpr, t0, t1, cap):
    out = []
    while t0 < t1:
        g, c = divmod(t0, tpr)
        if c == 0 and t1 - t0 >= tpr and tpr <= cap:
            left = (t1 - t0) // tpr
            n = -(-left // -(-left // (cap // tpr)))
            out.append((8 * g, 8 * n, 0, tpr * TILE))
            t0 += n * tpr
        else:
            left = min(tpr - c, t1 - t0)
            n = -(-left // -(-left // cap))
            out.append((8 * g, 8, c * TILE, n * TILE))
            t0 += n
    return out


def _units(rows, cols, unit):
    tpr = cols // TILE
    total = rows // 8 * tpr
    return [_rects(tpr, a, min(a + unit, total), 20) for a in range(0, total, unit)]


def _strided(lst, s):
    return [lst[i] for i in sorted(range(len(lst)), key=lambda i: (i % s, i // s))]


def _flat(lst):
    return [p for u in lst for p in u]


def _size(p):
    n = 1
    for v in p[1::2]:
        n *= v
    return n


def _merge(a, b):
    out, ia, ib, sa, sb = [], 0, 0, 0, 0
    while ia < len(a) or ib < len(b):
        if ib >= len(b) or (ia < len(a) and sa <= sb):
            out.append(a[ia] + (0,))
            sa += _size(a[ia][-1])
            ia += 1
        else:
            out.append(b[ib] + (1,))
            sb += _size(b[ib][-1])
            ib += 1
    return out


def _split(jobs, n):
    total = sum(_size(j[-2]) for j in jobs)
    out, acc = [[] for _ in range(n)], 0
    for j in jobs:
        out[min(n - 1, acc * n // total)].append(j)
        acc += _size(j[-2])
    return out


def _kv_pieces(n, rows):
    return [(8 * (g + r), 8 * min(n, rows - r), c, 512) for g in range(0, DH // 8, rows)
            for c in range(0, W, 512) for r in range(0, rows, n)]


def _runs(groups, r0, r1, c0, c1, n, rot=1):
    rs = _strided(list(range(r0, r1, 8)), (r1 - r0) // 8 // rot)
    return [(a, min(n, groups - a), r, 8, c, 512) for i in range(0, len(rs), rot) for c in range(c0, c1, 512)
            for r in rs[i:i + rot] for a in range(0, groups, n)]


def make_kernel(kv=(5, 24, 5, 24), wq=(5, 2, 1), wo=(8, 4, 1), w13=(4, 4, 1), w2=1,
                w2ch=((0, 0, 4), (1, 0, 4), (2, 0, 2), (2, 2, 2)), nq=4, xpos=0, R=4, NC=2, nobounds=True, rot=0,
                hplan=((0,), (1,), (2, 3)), gplan=((4,), (5,), (6,))):
    GQ, GO, G13 = wq[0], wo[0], w13[0]
    RQ, RO, R13 = D // GQ, H * DH // GO, D // G13
    HPG = H // GO
    FC = 512
    N13, N2 = F // FC, len(w2ch)
    A2, J2 = 4, F // 512
    kp, vp = _kv_pieces(kv[0], kv[1]), _kv_pieces(kv[2], kv[3])
    vp = vp[rot:] + vp[:rot]

    wqp = [_runs(GQ, t * RQ // 2, (t + 1) * RQ // 2, 0, H * DH, *wq[1:]) for t in range(2)]
    u = _units(RO, D, 4)
    u = _strided(u, len(u) // wo[2])
    wop = [[(a, wo[1]) + rect for blk in u for a in range(t * GO // 2, (t + 1) * GO // 2, wo[1]) for rect in blk]
           for t in range(2)]

    def kernel(x_hbm, kt_hbm, vt_hbm, wq_hbm, wo_hbm, w1_hbm, w3_hbm, w2_hbm, o_hbm,
               x_v, wq_v, q_v, kv_v, wo_v, w13_v, w2_v, o_v, sem_o):

        def body(sem_w, sem_kv, sem_w13, sem_w2):
            def issue(jobs):
                for (src, dst, sem, p, thread) in jobs:
                    idx = tuple(pl.ds(p[i], p[i + 1]) for i in range(0, len(p), 2))
                    pltpu.make_async_copy(src.at[idx], dst.at[idx], sem).start(priority=thread)

            def wait_all(ref, sem):
                pltpu.make_async_copy(ref, ref, sem).wait()

            def head_jobs(h, slot):
                return _merge(*[[(hbm.at[h, :, pl.ds(SK - W, W)], kv_v.at[slot, i], sem_kv.at[slot], p) for p in pieces]
                                for i, (hbm, pieces) in enumerate(((kt_hbm, kp), (vt_hbm, vp)))])

            def wait_part(slot, i, n):
                wait_all(kv_v.at[slot, :, :, pl.ds(i * (W // n), W // n)], sem_kv.at[slot])

            jobs = _merge(*[[(wq_hbm, wq_v, sem_w, p) for p in half] for half in wqp])
            issue(jobs[:xpos])
            pltpu.make_async_copy(x_hbm, x_v, sem_w).start()
            issue(jobs[xpos:])
            issue(_merge(*[[(wo_hbm, wo_v, sem_w, p) for p in half] for half in wop]))
            wait_all(x_v, sem_w)
            issue(head_jobs(0, 0))
            wait_all(wq_v, sem_w)
            wait_all(wo_v, sem_w)

            x32 = x_v[...].astype(F32)
            lnx = jnp.broadcast_to(_layernorm(x32), (8, D))
            QC = H // nq
            for c, group in enumerate(_split(_flat(head_jobs(h, h) for h in range(1, R - 1)), nq)):
                wq_c = wq_v[:, :, c * QC * DH:(c + 1) * QC * DH].reshape(D, QC * DH)
                qc = jnp.dot(lnx, wq_c, preferred_element_type=F32)
                for j in range(QC):
                    q_v[c * QC + j] = qc[:, j * DH:(j + 1) * DH]
                issue(group)
                wait_part(0, c, nq)

            def head(h, slot, nxt, attn, jobs):
                groups = _split(jobs, 2 * NC)

                def feed(i):
                    issue(groups[i])
                    if nxt is not None:
                        wait_part(nxt, i, 2 * NC)

                cols = [pl.ds(i * (W // NC), W // NC) for i in range(NC)]
                qh = q_v[h].astype(BF)
                s = []
                for i in range(NC):
                    s.append(jnp.dot(qh, kv_v[slot, 0, :, cols[i]], preferred_element_type=F32))
                    feed(i)
                s = _r(_r(jnp.concatenate(s, axis=1)) * SCALE)
                m = jnp.max(s, axis=-1, keepdims=True)
                e = _r(jnp.exp(_r(s - m)))
                l = _r(jnp.sum(e, axis=-1, keepdims=True))
                p = (e / l).astype(BF)
                o = None
                for i in range(NC):
                    o_ = lax.dot_general(p[:, i * (W // NC):(i + 1) * (W // NC)], kv_v[slot, 1, :, cols[i]],
                                         (((1,), (1,)), ((), ())), preferred_element_type=F32)
                    o = o_ if o is None else o + o_
                    if i < NC - 1:
                        feed(NC + i)
                row = (h % HPG) * DH
                if not isinstance(h, int):
                    row = pl.multiple_of(row, DH)
                attn = attn + jnp.dot(o.astype(BF), wo_v[h // HPG, pl.ds(row, DH), :], preferred_element_type=F32)
                feed(2 * NC - 1)
                return attn

            def step(h, attn):
                return head(h, h % R, (h + 1) % R, attn, head_jobs(h + R - 1, (h + R - 1) % R))

            attn = lax.fori_loop(0, H - R + 1, step, jnp.zeros((8, D), F32))

            wch = []
            for c in range(N13):
                pp = _runs(G13, 0, R13, c * FC, (c + 1) * FC, *w13[1:])
                wch.append(_merge([(w1_hbm, w13_v.at[0], sem_w13.at[c], p) for p in pp],
                                  [(w3_hbm, w13_v.at[1], sem_w13.at[c], p) for p in pp]))
            u2 = _units(128, D, 4)
            for c, (j, a, n) in enumerate(w2ch):
                wch.append(_merge(*[[(w2_hbm, w2_v, sem_w2.at[c], (a, n, j, 1) + rect)
                                     for rect in _flat(_strided(half, len(half) // w2))]
                                    for half in (u2[:len(u2) // 2], u2[len(u2) // 2:])]))
            for h, chunks in zip(range(H - R + 1, H), hplan, strict=True):
                attn = head(h, h % R, (h + 1) % R if h + 1 < H else None, attn, _flat(wch[c] for c in chunks))
            hres = _r(x32 + _r(attn))
            lnh = _layernorm(hres)
            hm = []
            for c in range(N13):
                cols = pl.ds(c * FC, FC)
                wait_all(w13_v.at[:, :, :, cols], sem_w13.at[c])
                gate = _r(jnp.dot(lnh, w13_v[0, :, :, cols].reshape(D, FC), preferred_element_type=F32))
                up = _r(jnp.dot(lnh, w13_v[1, :, :, cols].reshape(D, FC), preferred_element_type=F32))
                hm.append((_r(gate * _r(jax.nn.sigmoid(gate))) * up).astype(BF))
                issue(_flat(wch[i] for i in gplan[c]))
            hm = jnp.concatenate(hm, axis=1)
            out = None
            for c, (j, a, n) in enumerate(w2ch):
                wait_all(w2_v.at[pl.ds(a, n), pl.ds(j, 1)], sem_w2.at[c])
                hc = jnp.concatenate([hm[:, (i * J2 + j) * 128:(i * J2 + j + 1) * 128] for i in range(a, a + n)], axis=1)
                o_ = jnp.dot(hc, w2_v[a:a + n, j].reshape(n * 128, D), preferred_element_type=F32)
                out = o_ if out is None else out + o_
                for chunks in gplan[N13 + c:N13 + c + 1]:
                    issue(_flat(wch[i] for i in chunks))
            res = hres + _r(out)
            o_v[...] = res[0:1, :].astype(o_v.dtype)
            pltpu.make_async_copy(o_v, o_hbm, sem_o).start()

        dma = pltpu.SemaphoreType.DMA
        pl.run_scoped(body, dma(()), dma((R,)), dma((N13,)), dma((N2,)))
        pltpu.make_async_copy(o_v, o_hbm, sem_o).wait()

    @jax.jit
    def run(A_x, A_k_cache, A_v_cache, A_wq, A_wo, B_x, B_w1, B_w3, B_w2):
        del B_x
        x = A_x.reshape(1, D)
        kt = jnp.swapaxes(A_k_cache.reshape(H, SK, DH), 1, 2)
        vt = jnp.swapaxes(A_v_cache.reshape(H, SK, DH), 1, 2)
        out = pl.pallas_call(
            kernel,
            out_shape=jax.ShapeDtypeStruct((1, D), A_x.dtype),
            in_specs=[pl.BlockSpec(memory_space=pl.ANY)] * 8,
            out_specs=pl.BlockSpec(memory_space=pl.ANY),
            scratch_shapes=[
                pltpu.VMEM((1, D), BF),
                pltpu.VMEM((GQ, RQ, H * DH), BF),
                pltpu.VMEM((H, 8, DH), F32),
                pltpu.VMEM((R, 2, DH, W), BF),
                pltpu.VMEM((GO, RO, D), BF),
                pltpu.VMEM((2, G13, R13, F), BF),
                pltpu.VMEM((A2, J2, 128, D), BF),
                pltpu.VMEM((1, D), BF),
                pltpu.SemaphoreType.DMA(()),
            ],
            compiler_params=pltpu.CompilerParams(vmem_limit_bytes=64 * 1024 * 1024, disable_bounds_checks=nobounds),
        )(x, kt, vt, A_wq.reshape(GQ, RQ, H * DH), A_wo.reshape(GO, RO, D),
          B_w1.reshape(G13, R13, F), B_w3.reshape(G13, R13, F), B_w2.reshape(A2, J2, 128, D))
        return out.reshape(1, 1, D)

    return run


pallas_sequential_preLN__sliding_block_cached__glu_gated_swiglu__decode_kernel = make_kernel()
```

```python
import jax
import jax.numpy as jnp
import numpy as np
from jax import lax
import jax.experimental.pallas as pl
import jax.experimental.pallas.tpu as pltpu

H, DH, SK, D, F = 32, 192, 32768, 640, 1536
W = min(4096, max(256, SK // 4))
BF = jnp.bfloat16
F32 = jnp.float32


def _bf16_round(v):
    u = int(np.float32(v).view(np.uint32))
    u = (u + 0x7FFF + ((u >> 16) & 1)) & 0xFFFF0000
    return float(np.uint32(u).view(np.float32))


SCALE = _bf16_round(DH ** -0.5)
EPS = _bf16_round(1e-5)


def _r(x):
    return x.astype(BF).astype(F32)


def _layernorm(x32):
    m = jnp.mean(x32, axis=-1, keepdims=True)
    c = x32 - m
    v = jnp.mean(c * c, axis=-1, keepdims=True)
    num = _r(x32 - _r(m))
    den = _r(jnp.sqrt(_r(_r(v) + EPS)))
    return (num / den).astype(BF)


TILE = 128


def _rects(tpr, t0, t1, cap):
    out = []
    while t0 < t1:
        g, c = divmod(t0, tpr)
        if c == 0 and t1 - t0 >= tpr and tpr <= cap:
            left = (t1 - t0) // tpr
            n = -(-left // -(-left // (cap // tpr)))
            out.append((8 * g, 8 * n, 0, tpr * TILE))
            t0 += n * tpr
        else:
            left = min(tpr - c, t1 - t0)
            n = -(-left // -(-left // cap))
            out.append((8 * g, 8, c * TILE, n * TILE))
            t0 += n
    return out


def _units(rows, cols, unit):
    tpr = cols // TILE
    total = rows // 8 * tpr
    return [_rects(tpr, a, min(a + unit, total), 20) for a in range(0, total, unit)]


def _strided(lst, s):
    return [lst[i] for i in sorted(range(len(lst)), key=lambda i: (i % s, i // s))]


def _flat(lst):
    return [p for u in lst for p in u]


def _size(p):
    n = 1
    for v in p[1::2]:
        n *= v
    return n


def _merge(a, b):
    out, ia, ib, sa, sb = [], 0, 0, 0, 0
    while ia < len(a) or ib < len(b):
        if ib >= len(b) or (ia < len(a) and sa <= sb):
            out.append(a[ia] + (0,))
            sa += _size(a[ia][-1])
            ia += 1
        else:
            out.append(b[ib] + (1,))
            sb += _size(b[ib][-1])
            ib += 1
    return out


def _split(jobs, n):
    total = sum(_size(j[-2]) for j in jobs)
    out, acc = [[] for _ in range(n)], 0
    for j in jobs:
        out[min(n - 1, acc * n // total)].append(j)
        acc += _size(j[-2])
    return out


def _kv_pieces(n, rows):
    return [(8 * (g + r), 8 * min(n, rows - r), c, 512) for g in range(0, DH // 8, rows)
            for c in range(0, W, 512) for r in range(0, rows, n)]


def _runs(groups, r0, r1, c0, c1, n, rot=1):
    rs = _strided(list(range(r0, r1, 8)), (r1 - r0) // 8 // rot)
    return [(a, min(n, groups - a), r, 8, c, 512) for i in range(0, len(rs), rot) for c in range(c0, c1, 512)
            for r in rs[i:i + rot] for a in range(0, groups, n)]


def make_kernel(kv=(5, 24, 5, 24), wq=(5, 2, 1), wo=(16, 2, 1), w13=(4, 2, 1), w2=(4, 4, 1),
                w2ch=(128, 128, 64, 64), nq=4, xpos=0, R=4, NC=2, nobounds=True, rot=0,
                hplan=((0,), (1,), (2, 3)), gplan=((4,), (5,), (6,))):
    GQ, GO, G13 = wq[0], wo[0], w13[0]
    RQ, RO, R13 = D // GQ, H * DH // GO, D // G13
    HPG = H // GO
    FC = 512
    N13, N2 = F // FC, len(w2ch)
    G2, R2 = w2[0], F // w2[0]
    w2off = [sum(w2ch[:i]) for i in range(N2)]
    kp, vp = _kv_pieces(kv[0], kv[1]), _kv_pieces(kv[2], kv[3])
    vp = vp[rot:] + vp[:rot]

    wqp = [_runs(GQ, t * RQ // 2, (t + 1) * RQ // 2, 0, H * DH, *wq[1:]) for t in range(2)]
    u = _units(RO, D, 4)
    u = _strided(u, len(u) // wo[2])
    wop = [[(a, wo[1]) + rect for blk in u for a in range(t * GO // 2, (t + 1) * GO // 2, wo[1]) for rect in blk]
           for t in range(2)]

    def kernel(x_hbm, kt_hbm, vt_hbm, wq_hbm, wo_hbm, w1_hbm, w3_hbm, w2_hbm, o_hbm,
               x_v, wq_v, q_v, kv_v, wo_v, w13_v, w2_v, o_v, sem_o):

        def body(sem_w, sem_kv, sem_w13, sem_w2):
            def issue(jobs):
                for (src, dst, sem, p, thread) in jobs:
                    idx = tuple(pl.ds(p[i], p[i + 1]) for i in range(0, len(p), 2))
                    pltpu.make_async_copy(src.at[idx], dst.at[idx], sem).start(priority=thread)

            def wait_all(ref, sem):
                pltpu.make_async_copy(ref, ref, sem).wait()

            def head_jobs(h, slot):
                return _merge(*[[(hbm.at[h, :, pl.ds(SK - W, W)], kv_v.at[slot, i], sem_kv.at[slot], p) for p in pieces]
                                for i, (hbm, pieces) in enumerate(((kt_hbm, kp), (vt_hbm, vp)))])

            def wait_part(slot, i, n):
                wait_all(kv_v.at[slot, :, :, pl.ds(i * (W // n), W // n)], sem_kv.at[slot])

            jobs = _merge(*[[(wq_hbm, wq_v, sem_w, p) for p in half] for half in wqp])
            issue(jobs[:xpos])
            pltpu.make_async_copy(x_hbm, x_v, sem_w).start()
            issue(jobs[xpos:])
            issue(_merge(*[[(wo_hbm, wo_v, sem_w, p) for p in half] for half in wop]))
            wait_all(x_v, sem_w)
            issue(head_jobs(0, 0))
            wait_all(wq_v, sem_w)
            wait_all(wo_v, sem_w)

            x32 = x_v[...].astype(F32)
            lnx = jnp.broadcast_to(_layernorm(x32), (8, D))
            QC = H // nq
            for c, group in enumerate(_split(_flat(head_jobs(h, h) for h in range(1, R - 1)), nq)):
                wq_c = wq_v[:, :, c * QC * DH:(c + 1) * QC * DH].reshape(D, QC * DH)
                qc = jnp.dot(lnx, wq_c, preferred_element_type=F32)
                for j in range(QC):
                    q_v[c * QC + j] = qc[:, j * DH:(j + 1) * DH]
                issue(group)
                wait_part(0, c, nq)

            def head(h, slot, nxt, attn, jobs):
                groups = _split(jobs, 2 * NC)

                def feed(i):
                    issue(groups[i])
                    if nxt is not None:
                        wait_part(nxt, i, 2 * NC)

                cols = [pl.ds(i * (W // NC), W // NC) for i in range(NC)]
                qh = q_v[h].astype(BF)
                s = []
                for i in range(NC):
                    s.append(jnp.dot(qh, kv_v[slot, 0, :, cols[i]], preferred_element_type=F32))
                    feed(i)
                s = _r(_r(jnp.concatenate(s, axis=1)) * SCALE)
                m = jnp.max(s, axis=-1, keepdims=True)
                e = _r(jnp.exp(_r(s - m)))
                l = _r(jnp.sum(e, axis=-1, keepdims=True))
                p = (e / l).astype(BF)
                o = None
                for i in range(NC):
                    o_ = lax.dot_general(p[:, i * (W // NC):(i + 1) * (W // NC)], kv_v[slot, 1, :, cols[i]],
                                         (((1,), (1,)), ((), ())), preferred_element_type=F32)
                    o = o_ if o is None else o + o_
                    if i < NC - 1:
                        feed(NC + i)
                row = (h % HPG) * DH
                if not isinstance(h, int):
                    row = pl.multiple_of(row, DH)
                attn = attn + jnp.dot(o.astype(BF), wo_v[h // HPG, pl.ds(row, DH), :], preferred_element_type=F32)
                feed(2 * NC - 1)
                return attn

            def step(h, attn):
                return head(h, h % R, (h + 1) % R, attn, head_jobs(h + R - 1, (h + R - 1) % R))

            attn = lax.fori_loop(0, H - R + 1, step, jnp.zeros((8, D), F32))

            wch = []
            for c in range(N13):
                pp = _runs(G13, 0, R13, c * FC, (c + 1) * FC, *w13[1:])
                wch.append(_merge([(w1_hbm, w13_v.at[0], sem_w13.at[c], p) for p in pp],
                                  [(w3_hbm, w13_v.at[1], sem_w13.at[c], p) for p in pp]))
            for c in range(N2):
                u2 = _units(w2ch[c], D, 4)
                wch.append(_merge(*[[(w2_hbm, w2_v, sem_w2.at[c], (a, w2[1], w2off[c] + r, nr, c0, nc))
                                     for blk in _strided(half, max(1, len(half) // w2[2]))
                                     for a in range(0, G2, w2[1]) for (r, nr, c0, nc) in blk]
                                    for half in (u2[:len(u2) // 2], u2[len(u2) // 2:])]))
            for h, chunks in zip(range(H - R + 1, H), hplan, strict=True):
                attn = head(h, h % R, (h + 1) % R if h + 1 < H else None, attn, _flat(wch[c] for c in chunks))
            hres = _r(x32 + _r(attn))
            lnh = _layernorm(hres)
            hm = []
            for c in range(N13):
                cols = pl.ds(c * FC, FC)
                wait_all(w13_v.at[:, :, :, cols], sem_w13.at[c])
                gate = _r(jnp.dot(lnh, w13_v[0, :, :, cols].reshape(D, FC), preferred_element_type=F32))
                up = _r(jnp.dot(lnh, w13_v[1, :, :, cols].reshape(D, FC), preferred_element_type=F32))
                hm.append((_r(gate * _r(jax.nn.sigmoid(gate))) * up).astype(BF))
                issue(_flat(wch[i] for i in gplan[c]))
            hm = jnp.concatenate(hm, axis=1)
            out = None
            for c in range(N2):
                r0, nr = w2off[c], w2ch[c]
                hc = jnp.concatenate([hm[:, g * R2 + r0:g * R2 + r0 + nr] for g in range(G2)], axis=1)
                wait_all(w2_v.at[:, pl.ds(r0, nr)], sem_w2.at[c])
                o_ = jnp.dot(hc, w2_v[:, r0:r0 + nr].reshape(G2 * nr, D), preferred_element_type=F32)
                out = o_ if out is None else out + o_
                for chunks in gplan[N13 + c:N13 + c + 1]:
                    issue(_flat(wch[i] for i in chunks))
            res = hres + _r(out)
            o_v[...] = res[0:1, :].astype(o_v.dtype)
            pltpu.make_async_copy(o_v, o_hbm, sem_o).start()

        dma = pltpu.SemaphoreType.DMA
        pl.run_scoped(body, dma(()), dma((R,)), dma((N13,)), dma((N2,)))
        pltpu.make_async_copy(o_v, o_hbm, sem_o).wait()

    @jax.jit
    def run(A_x, A_k_cache, A_v_cache, A_wq, A_wo, B_x, B_w1, B_w3, B_w2):
        del B_x
        x = A_x.reshape(1, D)
        kt = jnp.swapaxes(A_k_cache.reshape(H, SK, DH), 1, 2)
        vt = jnp.swapaxes(A_v_cache.reshape(H, SK, DH), 1, 2)
        out = pl.pallas_call(
            kernel,
            out_shape=jax.ShapeDtypeStruct((1, D), A_x.dtype),
            in_specs=[pl.BlockSpec(memory_space=pl.ANY)] * 8,
            out_specs=pl.BlockSpec(memory_space=pl.ANY),
            scratch_shapes=[
                pltpu.VMEM((1, D), BF),
                pltpu.VMEM((GQ, RQ, H * DH), BF),
                pltpu.VMEM((H, 8, DH), F32),
                pltpu.VMEM((R, 2, DH, W), BF),
                pltpu.VMEM((GO, RO, D), BF),
                pltpu.VMEM((2, G13, R13, F), BF),
                pltpu.VMEM((G2, R2, D), BF),
                pltpu.VMEM((1, D), BF),
                pltpu.SemaphoreType.DMA(()),
            ],
            compiler_params=pltpu.CompilerParams(vmem_limit_bytes=64 * 1024 * 1024, disable_bounds_checks=nobounds),
        )(x, kt, vt, A_wq.reshape(GQ, RQ, H * DH), A_wo.reshape(GO, RO, D),
          B_w1.reshape(G13, R13, F), B_w3.reshape(G13, R13, F), B_w2.reshape(G2, R2, D))
        return out.reshape(1, 1, D)

    return run


pallas_sequential_preLN__sliding_block_cached__glu_gated_swiglu__decode_kernel = make_kernel()
```

```python
import jax
import jax.numpy as jnp
import numpy as np
from jax import lax
import jax.experimental.pallas as pl
import jax.experimental.pallas.tpu as pltpu

H, DH, SK, D, F = 32, 192, 32768, 640, 1536
W = min(4096, max(256, SK // 4))
BF = jnp.bfloat16
F32 = jnp.float32


def _bf16_round(v):
    u = int(np.float32(v).view(np.uint32))
    u = (u + 0x7FFF + ((u >> 16) & 1)) & 0xFFFF0000
    return float(np.uint32(u).view(np.float32))


SCALE = _bf16_round(DH ** -0.5)
EPS = _bf16_round(1e-5)


def _r(x):
    return x.astype(BF).astype(F32)


def _layernorm(x32):
    m = jnp.mean(x32, axis=-1, keepdims=True)
    c = x32 - m
    v = jnp.mean(c * c, axis=-1, keepdims=True)
    num = _r(x32 - _r(m))
    den = _r(jnp.sqrt(_r(_r(v) + EPS)))
    return (num / den).astype(BF)


TILE = 128


def _units(rows, cols):
    tpr = cols // TILE
    out = []
    for t0 in range(0, rows // 8 * tpr, 4):
        g, c = divmod(t0, tpr)
        n = min(4, tpr - c)
        out.append([(8 * g, 8, c * TILE, n * TILE)] + ([(8 * g + 8, 8, 0, (4 - n) * TILE)] if n < 4 else []))
    return out


def _flat(lst):
    return [p for u in lst for p in u]


def _size(p):
    n = 1
    for v in p[1::2]:
        n *= v
    return n


def _merge(a, b):
    out, ia, ib, sa, sb = [], 0, 0, 0, 0
    while ia < len(a) or ib < len(b):
        if ib >= len(b) or (ia < len(a) and sa <= sb):
            out.append(a[ia] + (0,))
            sa += _size(a[ia][-1])
            ia += 1
        else:
            out.append(b[ib] + (1,))
            sb += _size(b[ib][-1])
            ib += 1
    return out


def _split(jobs, n):
    total = sum(_size(j[-2]) for j in jobs)
    out, acc = [[] for _ in range(n)], 0
    for j in jobs:
        out[min(n - 1, acc * n // total)].append(j)
        acc += _size(j[-2])
    return out


def _kv_pieces(n, rows):
    return [(8 * (g + r), 8 * min(n, rows - r), c, 512) for g in range(0, DH // 8, rows)
            for c in range(0, W, 512) for r in range(0, rows, n)]


def _runs(groups, r0, r1, c0, c1, n):
    return [(a, min(n, groups - a), r, 8, c, 512) for r in range(r0, r1, 8) for c in range(c0, c1, 512)
            for a in range(0, groups, n)]


def make_kernel(kv=(5, 24), wq=(5, 2), wo=(16, 2), w13=(4, 4), w2=(4, 4), w2ch=(128, 128, 64, 64), nq=4, R=4, NC=2,
                hplan=((0,), (1,), (2, 3)), gplan=((4,), (5,), (6,))):
    GQ, GO, G13 = wq[0], wo[0], w13[0]
    RQ, RO, R13 = D // GQ, H * DH // GO, D // G13
    HPG = H // GO
    FC = 512
    N13, N2 = F // FC, len(w2ch)
    G2, R2 = w2[0], F // w2[0]
    w2off = [sum(w2ch[:i]) for i in range(N2)]
    kvp = _kv_pieces(*kv)

    wqp = [_runs(GQ, t * RQ // 2, (t + 1) * RQ // 2, 0, H * DH, wq[1]) for t in range(2)]
    u = _units(RO, D)
    wop = [[(a, wo[1]) + rect for blk in u for a in range(t * GO // 2, (t + 1) * GO // 2, wo[1]) for rect in blk]
           for t in range(2)]

    def kernel(x_hbm, kt_hbm, vt_hbm, wq_hbm, wo_hbm, w1_hbm, w3_hbm, w2_hbm, o_hbm,
               x_v, wq_v, q_v, kv_v, wo_v, w13_v, w2_v, o_v, sem_o):

        def body(sem_w, sem_kv, sem_w13, sem_w2):
            def issue(jobs):
                for (src, dst, sem, p, thread) in jobs:
                    idx = tuple(pl.ds(p[i], p[i + 1]) for i in range(0, len(p), 2))
                    pltpu.make_async_copy(src.at[idx], dst.at[idx], sem).start(priority=thread)

            def wait_all(ref, sem):
                pltpu.make_async_copy(ref, ref, sem).wait()

            def head_jobs(h, slot):
                return _merge(*[[(hbm.at[h, :, pl.ds(SK - W, W)], kv_v.at[slot, i], sem_kv.at[slot], p) for p in kvp]
                                for i, hbm in enumerate((kt_hbm, vt_hbm))])

            def wait_part(slot, i, n):
                wait_all(kv_v.at[slot, :, :, pl.ds(i * (W // n), W // n)], sem_kv.at[slot])

            pltpu.make_async_copy(x_hbm, x_v, sem_w).start()
            issue(_merge(*[[(wq_hbm, wq_v, sem_w, p) for p in half] for half in wqp]))
            issue(_merge(*[[(wo_hbm, wo_v, sem_w, p) for p in half] for half in wop]))
            wait_all(x_v, sem_w)
            issue(head_jobs(0, 0))
            wait_all(wq_v, sem_w)
            wait_all(wo_v, sem_w)

            x32 = x_v[...].astype(F32)
            lnx = jnp.broadcast_to(_layernorm(x32), (8, D))
            QC = H // nq
            for c, group in enumerate(_split(_flat(head_jobs(h, h) for h in range(1, R - 1)), nq)):
                wq_c = wq_v[:, :, c * QC * DH:(c + 1) * QC * DH].reshape(D, QC * DH)
                qc = jnp.dot(lnx, wq_c, preferred_element_type=F32)
                for j in range(QC):
                    q_v[c * QC + j] = qc[:, j * DH:(j + 1) * DH]
                issue(group)
                wait_part(0, c, nq)

            def head(h, slot, nxt, attn, jobs):
                groups = _split(jobs, 2 * NC)

                def feed(i):
                    issue(groups[i])
                    if nxt is not None:
                        wait_part(nxt, i, 2 * NC)

                cols = [pl.ds(i * (W // NC), W // NC) for i in range(NC)]
                qh = q_v[h].astype(BF)
                s = []
                for i in range(NC):
                    s.append(jnp.dot(qh, kv_v[slot, 0, :, cols[i]], preferred_element_type=F32))
                    feed(i)
                s = _r(_r(jnp.concatenate(s, axis=1)) * SCALE)
                m = jnp.max(s, axis=-1, keepdims=True)
                e = _r(jnp.exp(_r(s - m)))
                l = _r(jnp.sum(e, axis=-1, keepdims=True))
                p = (e / l).astype(BF)
                o = None
                for i in range(NC):
                    o_ = lax.dot_general(p[:, i * (W // NC):(i + 1) * (W // NC)], kv_v[slot, 1, :, cols[i]],
                                         (((1,), (1,)), ((), ())), preferred_element_type=F32)
                    o = o_ if o is None else o + o_
                    if i < NC - 1:
                        feed(NC + i)
                row = (h % HPG) * DH
                if not isinstance(h, int):
                    row = pl.multiple_of(row, DH)
                attn = attn + jnp.dot(o.astype(BF), wo_v[h // HPG, pl.ds(row, DH), :], preferred_element_type=F32)
                feed(2 * NC - 1)
                return attn

            def step(h, attn):
                return head(h, h % R, (h + 1) % R, attn, head_jobs(h + R - 1, (h + R - 1) % R))

            attn = lax.fori_loop(0, H - R + 1, step, jnp.zeros((8, D), F32))

            wch = []
            for c in range(N13):
                pp = _runs(G13, 0, R13, c * FC, (c + 1) * FC, w13[1])
                wch.append(_merge([(w1_hbm, w13_v.at[0], sem_w13.at[c], p) for p in pp],
                                  [(w3_hbm, w13_v.at[1], sem_w13.at[c], p) for p in pp]))
            for c in range(N2):
                u2 = _units(w2ch[c], D)
                wch.append(_merge(*[[(w2_hbm, w2_v, sem_w2.at[c], (a, w2[1], w2off[c] + r, nr, c0, nc))
                                     for blk in half for a in range(0, G2, w2[1]) for (r, nr, c0, nc) in blk]
                                    for half in (u2[:len(u2) // 2], u2[len(u2) // 2:])]))
            for h, chunks in zip(range(H - R + 1, H), hplan, strict=True):
                attn = head(h, h % R, (h + 1) % R if h + 1 < H else None, attn, _flat(wch[c] for c in chunks))
            hres = _r(x32 + _r(attn))
            lnh = _layernorm(hres)
            hm = []
            for c in range(N13):
                cols = pl.ds(c * FC, FC)
                wait_all(w13_v.at[:, :, :, cols], sem_w13.at[c])
                gate = _r(jnp.dot(lnh, w13_v[0, :, :, cols].reshape(D, FC), preferred_element_type=F32))
                up = _r(jnp.dot(lnh, w13_v[1, :, :, cols].reshape(D, FC), preferred_element_type=F32))
                hm.append((_r(gate * _r(jax.nn.sigmoid(gate))) * up).astype(BF))
                issue(_flat(wch[i] for i in gplan[c]))
            hm = jnp.concatenate(hm, axis=1)
            out = None
            for c in range(N2):
                r0, nr = w2off[c], w2ch[c]
                hc = jnp.concatenate([hm[:, g * R2 + r0:g * R2 + r0 + nr] for g in range(G2)], axis=1)
                wait_all(w2_v.at[:, pl.ds(r0, nr)], sem_w2.at[c])
                o_ = jnp.dot(hc, w2_v[:, r0:r0 + nr].reshape(G2 * nr, D), preferred_element_type=F32)
                out = o_ if out is None else out + o_
                for chunks in gplan[N13 + c:N13 + c + 1]:
                    issue(_flat(wch[i] for i in chunks))
            res = hres + _r(out)
            o_v[...] = res[0:1, :].astype(o_v.dtype)
            pltpu.make_async_copy(o_v, o_hbm, sem_o).start()

        dma = pltpu.SemaphoreType.DMA
        pl.run_scoped(body, dma(()), dma((R,)), dma((N13,)), dma((N2,)))
        pltpu.make_async_copy(o_v, o_hbm, sem_o).wait()

    @jax.jit
    def run(A_x, A_k_cache, A_v_cache, A_wq, A_wo, B_x, B_w1, B_w3, B_w2):
        del B_x
        x = A_x.reshape(1, D)
        kt = jnp.swapaxes(A_k_cache.reshape(H, SK, DH), 1, 2)
        vt = jnp.swapaxes(A_v_cache.reshape(H, SK, DH), 1, 2)
        out = pl.pallas_call(
            kernel,
            out_shape=jax.ShapeDtypeStruct((1, D), A_x.dtype),
            in_specs=[pl.BlockSpec(memory_space=pl.ANY)] * 8,
            out_specs=pl.BlockSpec(memory_space=pl.ANY),
            scratch_shapes=[
                pltpu.VMEM((1, D), BF),
                pltpu.VMEM((GQ, RQ, H * DH), BF),
                pltpu.VMEM((H, 8, DH), F32),
                pltpu.VMEM((R, 2, DH, W), BF),
                pltpu.VMEM((GO, RO, D), BF),
                pltpu.VMEM((2, G13, R13, F), BF),
                pltpu.VMEM((G2, R2, D), BF),
                pltpu.VMEM((1, D), BF),
                pltpu.SemaphoreType.DMA(()),
            ],
            compiler_params=pltpu.CompilerParams(vmem_limit_bytes=64 * 1024 * 1024),
        )(x, kt, vt, A_wq.reshape(GQ, RQ, H * DH), A_wo.reshape(GO, RO, D),
          B_w1.reshape(G13, R13, F), B_w3.reshape(G13, R13, F), B_w2.reshape(G2, R2, D))
        return out.reshape(1, 1, D)

    return run


pallas_sequential_preLN__sliding_block_cached__glu_gated_swiglu__decode_kernel = make_kernel()
```
